```python
import os as _os
_os.environ.setdefault("JAX_PLATFORMS", "cpu")
import jax
import jax.numpy as jnp

def _softmax(x, axis=-1):
    return jax.nn.softmax(x, axis=axis)
def _gelu(x):
    return jax.nn.gelu(x, approximate=True)
def _silu(x):
    return jax.nn.silu(x)
def _sigmoid(x):
    return jax.nn.sigmoid(x)
def _layernorm(x, axis=-1, eps=1e-5):
    m = jnp.mean(x, axis=axis, keepdims=True)
    v = jnp.var(x, axis=axis, keepdims=True)
    return (x - m) / jnp.sqrt(v + eps)
def _scatter_add(tgt, idx, src, axis=0):
    return tgt.at[idx].add(src)
def _segment_sum(src, seg, n):
    return jax.ops.segment_sum(src, seg, n)
class _Rng:
    def __init__(self, key):
        self._k = key
    def _next(self):
        self._k, sub = jax.random.split(self._k)
        return sub
    def normal(self, shape):
        return jax.random.normal(self._next(), shape, dtype=jnp.bfloat16)
    def randint(self, lo, hi, shape):
        return jax.random.randint(self._next(), shape, lo, hi, dtype=jnp.int32)
    def uniform(self, shape, lo=0.0, hi=1.0):
        return jax.random.uniform(self._next(), shape, jnp.bfloat16, lo, hi)
    def permutation(self, n):
        return jax.random.permutation(self._next(), n)


kernel_name = 'standalone__gqa_softmax__near_ridge'

def setup_inputs():
    _rng = _Rng(jax.random.key(int.from_bytes(__import__("os").urandom(4), "little")))
    _w = (lambda a: (lambda t: t.astype(jnp.bfloat16) if jnp.issubdtype(t.dtype, jnp.floating) else t)(jnp.asarray(a)))
    B, Hq, Hkv, Sq, Sk, D = 8, 16, 8, 160, 2048, 256
    return {
        "q": _w((lambda *s: _rng.normal(s) * 0.05)(B, Hq, Sq, D)),
        "k": _w((lambda *s: _rng.normal(s) * 3.2)(B, Hkv, Sk, D)),
        "v": _w((lambda *s: _rng.normal(s) * 0.05)(B, Hkv, Sk, D)),
    }

def reference(q, k, v):
    B, Hq, Sq, D = q.shape
    Hkv = k.shape[1]
    rep = Hq // Hkv
    k = jnp.repeat(k, rep, axis=1)
    v = jnp.repeat(v, rep, axis=1)
    scale = D ** -0.5
    scores = jnp.einsum("bhqd,bhkd->bhqk", q, k) * scale
    p = _softmax(scores, axis=-1)
    return jnp.einsum("bhqk,bhkd->bhqd", p, v)
```

```python
import functools, math
import numpy as np
import jax, jax.numpy as jnp
from jax import lax
from jax.experimental import pallas as pl
from jax.experimental.pallas import tpu as pltpu

def gen_order(NC, kind):
    o = []
    if kind == 'A':
        for j in range(NC-1):
            o += [f'p{j}', f'v{j}', f'k{j}']
            if j == 0: o += ['d']
        o += [f'p{NC-1}', f'k{NC-1}', 'm', f'v{NC-1}', 'o']
    elif kind == 'B':
        o += ['p0','v0','d','k0']
        for j in range(1, NC):
            o += [f'k{j}']
            if j == NC-1: o += ['m']
            o += [f'p{j}', f'v{j}']
        o += ['o']
    elif kind == 'C':
        o += ['k0','d']
        for j in range(1, NC):
            o += [f'k{j}']
            if j == NC-1: o += ['m']
            o += [f'p{j-1}', f'v{j-1}']
        o += [f'p{NC-1}', f'v{NC-1}', 'o']
    elif kind == 'D':
        o += ['p0','v0','d']
        for j in range(1, NC):
            o += [f'p{j}', f'k{j-1}', f'v{j}']
        o.pop()
        o += [f'k{NC-1}', 'm', f'v{NC-1}', 'o']
    return o

def make_v7(C=256, NB=6, phases=((2,1,7),(2,2,None)), order='B', OB=1, flags=None, nobc=True, Glim=None, nodma=False, recip='pl', qsrc='val', msrc='val', dep=0, deprow=0, depcol=0):
    NCH = 2048 // C
    if isinstance(order, str): order = gen_order(NCH, order) if len(order) == 1 else order.split()
    W = max(p[1] for p in phases)
    def kern(q_hbm, k_hbm, v_hbm, o_hbm, kvq, obuf, s0, s1, m0, m1, sem_in, sem_o, *, G, M, Sk, D):
        c = (D ** -0.5) * math.log2(math.e)
        NC = Sk // C
        KO, VO, QO = 0, Sk, 2*Sk
        S = (s0, s1); Mx = (m0, m1)
        def cps_in(a, slot, kq=True, v=True):
            l = []
            if kq:
                l.append(pltpu.make_async_copy(k_hbm.at[a+1], kvq.at[slot, pl.ds(KO, Sk)], sem_in.at[slot]))
                l.append(pltpu.make_async_copy(q_hbm.at[a+1], kvq.at[slot, pl.ds(QO, M)], sem_in.at[slot]))
            if v:
                l.append(pltpu.make_async_copy(v_hbm.at[a], kvq.at[slot, pl.ds(VO, Sk)], sem_in.at[slot]))
            return l
        def wait_all(slot):
            pltpu.make_async_copy(kvq.at[slot], kvq.at[slot], sem_in.at[slot]).wait()
        def cp_o(g0, n):
            return pltpu.make_async_copy(obuf.at[pl.ds(g0, n)], o_hbm.at[pl.ds(g0, n)], sem_o)

        cbits = int(np.float32(c).view(np.int32))
        def cvec(dep_tile):
            t = pltpu.bitcast(dep_tile, jnp.int32)
            t = jnp.minimum(jnp.maximum(t, cbits), cbits)
            return pltpu.bitcast(t, jnp.float32)
        def block(a, par, slot, dma_fn, do_pv=True, do_qk=True, deprow=0):
            st = dict(mrun=None, lrun=None, acc=None, p={}, q=None, m=None, dep=None, deps=[])
            def getq():
                if qsrc == 'ref': return kvq[slot, QO:QO+M, :]
                if st['q'] is None: st['q'] = kvq[slot, QO:QO+M, :]
                return st['q']
            def getm():
                if msrc == 'ref': return jnp.tile(Mx[par][...], (1, C//128))
                if st['m'] is None: st['m'] = jnp.tile(Mx[par][...], (1, C//128))
                return st['m']
            for tok in order:
                t, j = tok[0], (int(tok[1:]) if len(tok) > 1 else None)
                if t == 'p' and do_pv:
                    d0 = S[par][:, j*C:(j+1)*C] - getm()
                    if dep and st['dep'] is not None:
                        p = jnp.exp2(d0 * jnp.tile(cvec(st['dep']), (M//8, C//128)))
                    else:
                        p = jnp.exp2(d0 * c)
                    for i in range(C//128):
                        tile = p[:, i*128:(i+1)*128]
                        st['lrun'] = tile if st['lrun'] is None else st['lrun'] + tile
                    st['p'][j] = p.astype(jnp.bfloat16)
                    if j == NC - 1:
                        l = jnp.sum(st['lrun'], axis=-1, keepdims=True)
                        st['inv'] = (1.0 / l) if recip == 'div' else pl.reciprocal(l, approx=False, full_range=False)
                elif t == 'v' and do_pv:
                    pv = jnp.dot(st['p'].pop(j), kvq[slot, VO+j*C:VO+(j+1)*C, :], preferred_element_type=jnp.float32)
                    st['acc'] = pv if st['acc'] is None else st['acc'] + pv
                elif t == 'k' and do_qk:
                    sc = lax.dot_general(getq(), kvq[slot, KO+j*C:KO+(j+1)*C, :], (((1,),(1,)),((),())), preferred_element_type=jnp.float32)
                    S[1-par][:, j*C:(j+1)*C] = sc
                    st['deps'].append(sc[deprow*8:deprow*8+8, depcol*128:depcol*128+128]); st['dep'] = st['deps'][-dep] if dep and len(st['deps']) >= dep else None
                    for i in range(C//128):
                        tile = sc[:, i*128:(i+1)*128]
                        st['mrun'] = tile if st['mrun'] is None else jnp.maximum(st['mrun'], tile)
                elif t == 'm' and do_qk:
                    Mx[1-par][...] = jnp.broadcast_to(jnp.max(st['mrun'], axis=-1, keepdims=True), m0.shape)
                elif t == 'o' and do_pv:
                    obuf[a] = (st['acc'] * st['inv']).astype(obuf.dtype)
                elif t == 'd':
                    dma_fn()

        def dma_starts(a):
            if nodma: return
            static = isinstance(a, int)
            def when(cond):
                if static: return (lambda f: f() if cond else None)
                return pl.when(cond)
            nxt = a + NB - W
            fs = (nxt % NB) if static else lax.rem(nxt, NB)
            @when(nxt < G - 1)
            def _():
                for cp in cps_in(nxt, fs): cp.start()
            @when(nxt == G - 1)
            def _():
                for cp in cps_in(G - 1, fs, kq=False): cp.start()
            if static:
                if a % OB == 0 and a >= OB: cp_o(a - OB, OB).start()
            elif OB == 1:
                @pl.when(a >= 1)
                def _(): cp_o(a - 1, 1).start()
            else:
                @pl.when(jnp.logical_and(lax.rem(a, OB) == 0, a >= OB))
                def _(): cp_o(a - OB, OB).start()

        if not nodma:
            for cp in cps_in(-1, NB - 1, v=False): cp.start()
            for a in range(NB - W):
                for cp in cps_in(a, a): cp.start()
            for cp in cps_in(-1, NB - 1, v=False): cp.wait()
        block(-1, 1, NB - 1, lambda: None, do_pv=False)

        def wait_step(a, slot):
            if nodma: return
            if isinstance(a, int) and a == G - 1:
                for cp in cps_in(a, slot, kq=False): cp.wait()
            else:
                wait_all(slot)
        a0 = 0
        for ph in phases:
            U, WU, n = ph[:3]
            dr = ph[3] if len(ph) > 3 else deprow
            assert U % 2 == 0 and U % WU == 0 and a0 % 2 == 0
            if n is None: n = (G - 1 - a0) // U
            def body(i, carry, a0=a0, U=U, WU=WU, dr=dr):
                for u in range(U):
                    a = a0 + i * U + u
                    if u % WU == 0:
                        for w in range(WU): wait_step(a + w, lax.rem(a + w, NB))
                    block(a, u % 2, lax.rem(a, NB), lambda: dma_starts(a), deprow=dr)
                return carry
            if n > 0: lax.fori_loop(0, n, body, 0)
            a0 += n * U
        for a in range(a0, G):
            wait_step(a, a % NB)
            block(a, a % 2, a % NB, lambda: dma_starts(a), do_qk=(a < G - 1), deprow=deprow)
        if not nodma:
            done = ((G - 1) // OB) * OB
            cp_o(done, G - done).start()
            for b in range(0, done, OB): cp_o(b, OB).wait()
            cp_o(done, G - done).wait()

    def fn(q, k, v):
        B, Hq, Sq, D = q.shape
        _, Hkv, Sk, _ = k.shape
        rep = Hq // Hkv
        G = B * Hkv
        M = rep * Sq
        q2 = q.reshape(G, M, D); k2 = k.reshape(G, Sk, D); v2 = v.reshape(G, Sk, D)
        out = pl.pallas_call(
            functools.partial(kern, G=(Glim or G), M=M, Sk=Sk, D=D),
            in_specs=[pl.BlockSpec(memory_space=pl.ANY)]*3,
            out_specs=pl.BlockSpec(memory_space=pl.ANY),
            out_shape=jax.ShapeDtypeStruct((G, M, D), q.dtype),
            scratch_shapes=[pltpu.VMEM((NB, 2*Sk + M, D), q.dtype),
                            pltpu.VMEM((G, M, D), q.dtype),
                            pltpu.VMEM((M, Sk), jnp.float32), pltpu.VMEM((M, Sk), jnp.float32),
                            pltpu.VMEM((M, 128), jnp.float32), pltpu.VMEM((M, 128), jnp.float32),
                            pltpu.SemaphoreType.DMA((NB,)), pltpu.SemaphoreType.DMA(())],
            compiler_params=pltpu.CompilerParams(vmem_limit_bytes=100*1024*1024, flags=flags, disable_bounds_checks=nobc),
        )(q2, k2, v2)
        return out.reshape(B, Hq, Sq, D)
    return fn


_impl = make_v7(256, 8, ((2, 1, 7, 20), (2, 2, None, 20)), 'B', msrc='ref', dep=1, deprow=20)


@jax.jit
def pallas_standalone__gqa_softmax__near_ridge_kernel(q, k, v):
    return _impl(q, k, v)
```

```python
import functools
import math

import numpy as np
import jax
import jax.numpy as jnp
from jax import lax
from jax.experimental import pallas as pl
from jax.experimental.pallas import tpu as pltpu

_C = 256
_NB = 8
_W = 2
_NSPLIT = 3
_N1 = 2
_OSTART = 30
_ROW = 20


def _order(nc):
    o = ["p0", "v0", "k0"]
    for j in range(1, nc):
        o.append(f"k{j}")
        if j == nc - 1:
            o.append("m")
        o += [f"p{j}", f"v{j}"]
        if j == 1:
            o.append("d")
    return o + ["o"]


def _kernel(q_hbm, k_hbm, v_hbm, o_hbm, kvq, obuf, s0, s1, m0, m1, sem_in, sem_h, sem_o,
            *, G, M, Sk, D):
    C, NB, W = _C, _NB, _W
    NC = Sk // C
    H = Sk // 2
    KO, VO, QO = 0, Sk, 2 * Sk
    S, Mx = (s0, s1), (m0, m1)
    order = _order(NC)
    c = (D ** -0.5) * math.log2(math.e)
    cbits = int(np.float32(c).view(np.int32))

    def cps_in(a, slot, kq=True):
        l = []
        if kq:
            l.append(pltpu.make_async_copy(k_hbm.at[a + 1], kvq.at[slot, pl.ds(KO, Sk)], sem_in.at[slot]))
            l.append(pltpu.make_async_copy(q_hbm.at[a + 1], kvq.at[slot, pl.ds(QO, M)], sem_in.at[slot]))
        l.append(pltpu.make_async_copy(v_hbm.at[a], kvq.at[slot, pl.ds(VO, Sk)], sem_in.at[slot]))
        return l

    def cps_half(a, slot, h, v=True):
        sem = sem_in.at[slot] if h == 0 else sem_h.at[slot]
        l = []
        if h == 0:
            l.append(pltpu.make_async_copy(q_hbm.at[a + 1], kvq.at[slot, pl.ds(QO, M)], sem))
        l.append(pltpu.make_async_copy(k_hbm.at[a + 1, pl.ds(h * H, H)],
                                       kvq.at[slot, pl.ds(KO + h * H, H)], sem))
        if v:
            l.append(pltpu.make_async_copy(v_hbm.at[a, pl.ds(h * H, H)],
                                           kvq.at[slot, pl.ds(VO + h * H, H)], sem))
        return l

    def starts(l):
        for cp in l:
            cp.start()

    def waits(l):
        for cp in l:
            cp.wait()

    def wait_slot(slot):
        pltpu.make_async_copy(kvq.at[slot], kvq.at[slot], sem_in.at[slot]).wait()

    def cp_o(g0, n):
        return pltpu.make_async_copy(obuf.at[pl.ds(g0, n)], o_hbm.at[pl.ds(g0, n)], sem_o)

    def c_after(tile):
        t = pltpu.bitcast(tile, jnp.int32)
        t = jnp.minimum(jnp.maximum(t, cbits), cbits)
        return pltpu.bitcast(t, jnp.float32)

    def fold(op, run, x):
        for i in range(C // 128):
            tile = x[:, i * 128:(i + 1) * 128]
            run = tile if run is None else op(run, tile)
        return run

    def block(a, par, slot, dma_fn, do_pv=True, do_qk=True, carry=None, mid=None):
        carry = {} if carry is None else carry
        q = mrun = lrun = acc = inv = last = None
        ps = {}
        for tok in order:
            t, j = tok[0], (int(tok[1:]) if len(tok) > 1 else None)
            if mid is not None and t == "k" and j == NC // 2:
                mid()
            if t == "p" and do_pv:
                d0 = S[par][:, j * C:(j + 1) * C] - jnp.tile(Mx[par][...], (1, C // 128))
                src = last if last is not None else carry.get("sc")
                if src is None:
                    p = jnp.exp2(d0 * c)
                else:
                    cv = c_after(src[_ROW * 8:_ROW * 8 + 8, 0:128])
                    p = jnp.exp2(d0 * jnp.tile(cv, (M // 8, C // 128)))
                lrun = fold(jnp.add, lrun, p)
                ps[j] = p.astype(jnp.bfloat16)
                if j == NC - 1:
                    l = jnp.sum(lrun, axis=-1, keepdims=True)
                    inv = pl.reciprocal(l, approx=False, full_range=False)
            elif t == "v" and do_pv:
                pv = jnp.dot(ps.pop(j), kvq[slot, VO + j * C:VO + (j + 1) * C, :],
                             preferred_element_type=jnp.float32)
                acc = pv if acc is None else acc + pv
            elif t == "k" and do_qk:
                if q is None:
                    q = kvq[slot, QO:QO + M, :]
                sc = lax.dot_general(q, kvq[slot, KO + j * C:KO + (j + 1) * C, :],
                                     (((1,), (1,)), ((), ())), preferred_element_type=jnp.float32)
                S[1 - par][:, j * C:(j + 1) * C] = sc
                last = sc
                if j == NC - 1:
                    carry["sc"] = sc
                mrun = fold(jnp.maximum, mrun, sc)
            elif t == "m" and do_qk:
                Mx[1 - par][...] = jnp.broadcast_to(jnp.max(mrun, axis=-1, keepdims=True), m0.shape)
            elif t == "o" and do_pv:
                obuf[a] = (acc * inv).astype(obuf.dtype)
            elif t == "d":
                dma_fn()

    def dma_starts(a):
        static = isinstance(a, int)

        def when(cond):
            if static:
                return lambda f: f() if cond else None
            return pl.when(cond)

        both = (lambda x, y: x and y) if static else jnp.logical_and
        nxt = a + NB - W
        fs = (nxt % NB) if static else lax.rem(nxt, NB)

        @when(nxt < G - 1)
        def _():
            starts(cps_in(nxt, fs))

        @when(nxt == G - 1)
        def _():
            starts(cps_in(G - 1, fs, kq=False))

        @when(both(a >= _OSTART, a <= 2 * _OSTART - 2))
        def _():
            cp_o(2 * (a - _OSTART), 2).start()

        @when(a > 2 * _OSTART - 2)
        def _():
            cp_o(a - 1, 1).start()

    for h in (0, 1):
        starts(cps_half(-1, NB - 1, h, v=False))
    for a in range(NB - W):
        if a < _NSPLIT:
            for h in (0, 1):
                starts(cps_half(a, a, h))
        else:
            starts(cps_in(a, a))
    waits(cps_half(-1, NB - 1, 0, v=False))
    block(-1, 1, NB - 1, lambda: None, do_pv=False,
          mid=lambda: waits(cps_half(-1, NB - 1, 1, v=False)))
    for a in range(_NSPLIT):
        waits(cps_half(a, a, 0))
        block(a, a % 2, a, lambda a=a: dma_starts(a), mid=lambda a=a: waits(cps_half(a, a, 1)))

    a0 = _NSPLIT
    for wu, n in ((1, _N1), (2, None)):
        if n is None:
            n = (G - 1 - a0) // 2

        def body(i, _, a0=a0, wu=wu):
            cr = {}
            for u in range(2):
                a = a0 + i * 2 + u
                if u % wu == 0:
                    cr.clear()
                    for w in range(wu):
                        wait_slot(lax.rem(a + w, NB))
                block(a, (a0 + u) % 2, lax.rem(a, NB), lambda a=a: dma_starts(a), carry=cr)
            return 0

        lax.fori_loop(0, n, body, 0)
        a0 += n * 2
    for a in range(a0, G):
        if a == G - 1:
            waits(cps_in(a, a % NB, kq=False))
        else:
            wait_slot(a % NB)
        block(a, a % 2, a % NB, lambda a=a: dma_starts(a), do_qk=(a < G - 1))
    cp_o(G - 1, 1).start()
    pltpu.make_async_copy(obuf, obuf, sem_o).wait()


@jax.jit
def pallas_standalone__gqa_softmax__near_ridge_kernel(
    q: jax.Array,
    k: jax.Array,
    v: jax.Array,
):
    B, Hq, Sq, D = q.shape
    _, Hkv, Sk, _ = k.shape
    G = B * Hkv
    M = (Hq // Hkv) * Sq
    assert Sk % (2 * _C) == 0 and D % 128 == 0 and M % 16 == 0 and M >= 8 * (_ROW + 1)
    assert G >= 2 * _OSTART and G > _NSPLIT + 2 * _N1 + _NB
    out = pl.pallas_call(
        functools.partial(_kernel, G=G, M=M, Sk=Sk, D=D),
        in_specs=[pl.BlockSpec(memory_space=pl.ANY)] * 3,
        out_specs=pl.BlockSpec(memory_space=pl.ANY),
        out_shape=jax.ShapeDtypeStruct((G, M, D), q.dtype),
        scratch_shapes=[
            pltpu.VMEM((_NB, 2 * Sk + M, D), q.dtype),
            pltpu.VMEM((G, M, D), q.dtype),
            pltpu.VMEM((M, Sk), jnp.float32), pltpu.VMEM((M, Sk), jnp.float32),
            pltpu.VMEM((M, 128), jnp.float32), pltpu.VMEM((M, 128), jnp.float32),
            pltpu.SemaphoreType.DMA((_NB,)), pltpu.SemaphoreType.DMA((_NB,)),
            pltpu.SemaphoreType.DMA(()),
        ],
        compiler_params=pltpu.CompilerParams(
            vmem_limit_bytes=100 * 1024 * 1024, disable_bounds_checks=True),
    )(q.reshape(G, M, D), k.reshape(G, Sk, D), v.reshape(G, Sk, D))
    return out.reshape(B, Hq, Sq, D)
```
